```python
import os as _os
_os.environ.setdefault("JAX_PLATFORMS", "cpu")
import jax
import jax.numpy as jnp

def _softmax(x, axis=-1):
    return jax.nn.softmax(x, axis=axis)
def _gelu(x):
    return jax.nn.gelu(x, approximate=True)
def _silu(x):
    return jax.nn.silu(x)
def _sigmoid(x):
    return jax.nn.sigmoid(x)
def _layernorm(x, axis=-1, eps=1e-5):
    m = jnp.mean(x, axis=axis, keepdims=True)
    v = jnp.var(x, axis=axis, keepdims=True)
    return (x - m) / jnp.sqrt(v + eps)
def _scatter_add(tgt, idx, src, axis=0):
    return tgt.at[idx].add(src)
def _segment_sum(src, seg, n):
    return jax.ops.segment_sum(src, seg, n)
class _Rng:
    def __init__(self, key):
        self._k = key
    def _next(self):
        self._k, sub = jax.random.split(self._k)
        return sub
    def normal(self, shape):
        return jax.random.normal(self._next(), shape, dtype=jnp.bfloat16)
    def randint(self, lo, hi, shape):
        return jax.random.randint(self._next(), shape, lo, hi, dtype=jnp.int32)
    def uniform(self, shape, lo=0.0, hi=1.0):
        return jax.random.uniform(self._next(), shape, jnp.bfloat16, lo, hi)
    def permutation(self, n):
        return jax.random.permutation(self._next(), n)


kernel_name = 'standalone__se_block__vision'

def setup_inputs():
    _rng = _Rng(jax.random.key(int.from_bytes(__import__("os").urandom(4), "little")))
    _w = (lambda a: (lambda t: t.astype(jnp.bfloat16) if jnp.issubdtype(t.dtype, jnp.floating) else t)(jnp.asarray(a)))
    H = W = 384
    C = 192; r = max(C // 16, 4)
    return {
        "x": _w((lambda *s: _rng.normal(s) * 0.8)(1, H, W, C)),
        "w_down": _w((lambda *s: _rng.normal(s) * 0.8)(C, r)),
        "w_up": _w((lambda *s: _rng.normal(s) * 0.8)(r, C)),
    }

def reference(x, w_down, w_up):
    s = x.mean(axis=(1, 2))
    s = _sigmoid(_silu(s @ w_down) @ w_up)
    return x * s[:, None, None, :]
```

```python
import jax
import jax.numpy as jnp
from jax import lax
import jax.experimental.pallas as pl
import jax.experimental.pallas.tpu as pltpu

_STREAMS = 6
_PIECE = 48
_READ_ROWS = (12, 24, 14, 7, 4, 2, 1)
_READ_DEPTH = 2


@jax.jit
def pallas_standalone__se_block__vision_kernel(
    x: jax.Array,
    w_down: jax.Array,
    w_up: jax.Array,
):
    _, H, W, C = x.shape
    R = w_up.shape[0]
    S, HS = _STREAMS, H // _STREAMS
    f32 = jnp.float32
    starts = [sum(_READ_ROWS[:i]) for i in range(len(_READ_ROWS))]
    nr, nsem = len(_READ_ROWS), _READ_DEPTH + 1

    def kernel(x_hbm, wd_hbm, wu_hbm, o_hbm, buf, wd_v, wu_v, s_v, rsem, wsem, msem):
        def rd(i):
            idx = (slice(None), pl.ds(starts[i], _READ_ROWS[i]))
            return pltpu.make_async_copy(x_hbm.at[idx], buf.at[idx], rsem.at[i % nsem])

        for i in range(_READ_DEPTH):
            rd(i).start()
        cwd = pltpu.make_async_copy(wd_hbm, wd_v, msem.at[0])
        cwu = pltpu.make_async_copy(wu_hbm, wu_v, msem.at[1])
        cwd.start()
        cwu.start()
        cwd.wait()
        cwu.wait()
        eye = (lax.broadcasted_iota(jnp.int32, (C, C), 0)
               == lax.broadcasted_iota(jnp.int32, (C, C), 1)).astype(jnp.bfloat16)
        nt = (((1,), (1,)), ((), ()))
        wdT = lax.dot_general(eye, wd_v[...], nt, preferred_element_type=f32) * (1.0 / (H * W))
        wuT = lax.dot_general(eye, wu_v[...], nt, preferred_element_type=f32)

        acc = jnp.zeros((C, 128), f32)
        for i in range(nr):
            rd(i).wait()
            if i + _READ_DEPTH < nr:
                rd(i + _READ_DEPTH).start()

            def body(t, acc, h0=starts[i]):
                for a in range(S):
                    v = buf[a, h0 + t].astype(f32)
                    acc = acc + ((v[:, 0:128] + v[:, 128:256]) + v[:, 256:384])
                return acc

            acc = lax.fori_loop(0, _READ_ROWS[i], body, acc)

        m = jnp.sum(acc, axis=1, keepdims=True)
        z = jnp.sum(m * wdT, axis=0, keepdims=True)
        hid = z * jax.nn.sigmoid(z)
        y = jnp.sum(wuT * hid, axis=1, keepdims=True)
        s_v[...] = jnp.broadcast_to(jax.nn.sigmoid(y), (C, 128))

        def wbody(h, _):
            for c0 in range(0, C, _PIECE):
                sc = s_v[c0:c0 + _PIECE, :]
                sc = jnp.concatenate([sc, sc, sc], axis=1)
                for a in range(S):
                    v = buf[a, h, c0:c0 + _PIECE, :].astype(f32)
                    buf[a, h, c0:c0 + _PIECE, :] = (v * sc).astype(jnp.bfloat16)
                idx = (slice(None), pl.ds(h, 1), pl.ds(c0, _PIECE))
                pltpu.make_async_copy(buf.at[idx], o_hbm.at[idx], wsem).start()
            return 0

        lax.fori_loop(0, HS, wbody, 0)
        pltpu.make_async_copy(buf, o_hbm, wsem).wait()

    xt = jnp.transpose(x.reshape(S, HS, W, C), (0, 1, 3, 2))
    out = pl.pallas_call(
        kernel,
        in_specs=[pl.BlockSpec(memory_space=pltpu.HBM)] * 3,
        out_specs=pl.BlockSpec(memory_space=pltpu.HBM),
        out_shape=jax.ShapeDtypeStruct((S, HS, C, W), x.dtype),
        scratch_shapes=[
            pltpu.VMEM((S, HS, C, W), x.dtype),
            pltpu.VMEM((R, C), w_down.dtype),
            pltpu.VMEM((R, C), w_up.dtype),
            pltpu.VMEM((C, 128), f32),
            pltpu.SemaphoreType.DMA((nsem,)),
            pltpu.SemaphoreType.DMA(()),
            pltpu.SemaphoreType.DMA((2,)),
        ],
        compiler_params=pltpu.CompilerParams(vmem_limit_bytes=100 * 2**20),
    )(xt, w_down.T, w_up)
    return jnp.transpose(out, (0, 1, 3, 2)).reshape(1, H, W, C)
```

```python
import jax
import jax.numpy as jnp
from jax import lax
import jax.experimental.pallas as pl
import jax.experimental.pallas.tpu as pltpu

_LANES = 128
_SUBLANES = 8
_PACKED = 16

_REGIONS = 6
_UNITS_PER_WRITE = 3
_READ_REGIONS = (3, 2)
_READ_WIDE_ROWS = (19, 4, 1)
_READ_TAIL_ROWS = (20, 3, 1)


def _tree_sum(terms):
    terms = list(terms)
    while len(terms) > 1:
        terms = [
            terms[i] + terms[i + 1] if i + 1 < len(terms) else terms[i]
            for i in range(0, len(terms), 2)
        ]
    return terms[0]


def _read_plan(rows, units):
    last = _REGIONS - 1
    split = rows - sum(_READ_TAIL_ROWS)
    assert sum(_READ_REGIONS) == last and split > 0
    assert sum(_READ_WIDE_ROWS) == sum(_READ_TAIL_ROWS)
    head, tail = [], []
    a = 0
    for n in _READ_REGIONS:
        head.append((a, n, 0, rows, 0, units))
        a += n
    head.append((last, 1, 0, split, 0, units))
    h = split
    for n in _READ_WIDE_ROWS:
        head.append((last, 1, h, n, 0, units - 1))
        h += n
    h = split
    for n in _READ_TAIL_ROWS:
        tail.append((last, 1, h, n, units - 1, 1))
        h += n
    return head, tail


def _se_kernel(x_hbm, wd_hbm, wu_hbm, o_hbm,
               buf, wd_ref, wu_ref, wd_t, wd_splat, wu_splat, s_ref, write_sem):
    f32 = jnp.float32
    regions, rows, units, unit_rows, _ = buf.shape
    rank, channels = wu_ref.shape
    rank_pad = wd_splat.shape[1]
    vregs = unit_rows // _PACKED
    groups = 2 * units
    inv_n = 1.0 / (regions * rows * vregs * _LANES)
    head, tail = _read_plan(rows, units)
    reads = head + tail

    def groups_of(p):
        return (2 * p) // vregs, (2 * p + 1) // vregs

    def body(read_sems, weight_sems):
        def read(i):
            a0, na, h0, nh, u0, nu = reads[i]
            idx = (pl.ds(a0, na), pl.ds(h0, nh), pl.ds(u0, nu))
            return pltpu.make_async_copy(x_hbm.at[idx], buf.at[idx], read_sems.at[i])

        for i in range(len(reads)):
            read(i).start(priority=1)
        wd_copy = pltpu.make_async_copy(wd_hbm, wd_ref, weight_sems.at[0])
        wu_copy = pltpu.make_async_copy(wu_hbm, wu_ref, weight_sems.at[1])
        wd_copy.start()
        wu_copy.start()
        wd_copy.wait()
        wu_copy.wait()

        eye = (
            lax.broadcasted_iota(jnp.int32, (channels, channels), 0)
            == lax.broadcasted_iota(jnp.int32, (channels, channels), 1)
        ).astype(wd_ref.dtype)

        def transposed(w_ref):
            return lax.dot_general(
                eye, w_ref[...], (((1,), (1,)), ((), ())), preferred_element_type=f32
            )

        wd_t[...] = jnp.zeros_like(wd_t)
        wd_t[:, 0:rank] = transposed(wd_ref) * inv_n
        wd_splat[...] = jnp.zeros_like(wd_splat)
        wd = wd_ref[...].astype(f32) * inv_n
        for k in range(_PACKED):
            c = channels - _PACKED + k
            wd_splat[k, 0:rank, :] = jnp.broadcast_to(wd[:, c:c + 1], (rank, _LANES))
        wu_t = transposed(wu_ref)
        for r in range(rank):
            column = jnp.broadcast_to(wu_t[:, r:r + 1], (channels, _LANES))
            wu_splat[:, r] = column.reshape(units, _PACKED, _LANES)

        def add_units(acc, a, h, u0, nu):
            acc = dict(acc)
            for u in range(u0, u0 + nu):
                for p in range(vregs):
                    v = buf[a, h, u, pl.ds(_PACKED * p, _PACKED), :].astype(f32)
                    lo, hi = groups_of(p)
                    acc[2 * u + lo] += v[:_SUBLANES]
                    acc[2 * u + hi] += v[_SUBLANES:]
            return acc

        def consume(acc, i):
            a0, na, h0, nh, u0, nu = reads[i]
            step = min(nh, max(units // nu, 1))
            while nh % step:
                step -= 1

            def region(a, acc):
                def chunk(j, acc):
                    for k in range(step):
                        acc = add_units(acc, a, h0 + j * step + k, u0, nu)
                    return acc

                if nh == step:
                    return chunk(0, acc)
                return lax.fori_loop(0, nh // step, chunk, acc)

            read(i).wait()
            if na == 1:
                return region(a0, acc)
            return lax.fori_loop(a0, a0 + na, region, acc)

        acc = {g: jnp.zeros((_SUBLANES, _LANES), f32) for g in range(groups)}
        for i in range(len(head)):
            acc = consume(acc, i)

        z = _tree_sum(
            jnp.sum(acc[g], axis=1, keepdims=True) * wd_t[pl.ds(_SUBLANES * g, _SUBLANES), :]
            for g in range(groups - 2)
        )
        z = jnp.sum(z, axis=0, keepdims=True)
        diagonal = lax.broadcasted_iota(
            jnp.int32, (rank_pad, _LANES), 0
        ) == lax.broadcasted_iota(jnp.int32, (rank_pad, _LANES), 1)
        z = jnp.sum(jnp.where(diagonal, z, 0.0), axis=1, keepdims=True)
        z = jnp.broadcast_to(z, (rank_pad, _LANES))

        acc = {g: acc[g] for g in (groups - 2, groups - 1)}
        for i in range(len(head), len(reads)):
            acc = consume(acc, i)

        sums = jnp.concatenate([acc[groups - 2], acc[groups - 1]], axis=0)
        sums = jnp.broadcast_to(jnp.sum(sums, axis=1, keepdims=True), (_PACKED, _LANES))
        terms = [
            wd_splat[k] * jnp.broadcast_to(sums[k:k + 1, :], (rank_pad, _LANES))
            for k in range(_PACKED)
        ]
        terms[0] = terms[0] + z
        z = _tree_sum(terms)
        hidden = z * jax.nn.sigmoid(z)
        hidden = [
            jnp.broadcast_to(hidden[r:r + 1, :], (_PACKED, _LANES)) for r in range(rank)
        ]

        def scale(h, u, s):
            halves = (s[:_SUBLANES], s[_SUBLANES:])
            per_vreg = [
                jnp.concatenate([halves[g] for g in groups_of(p)], axis=0)
                for p in range(vregs)
            ]
            for a in range(regions):
                for p in range(vregs):
                    sl = pl.ds(_PACKED * p, _PACKED)
                    v = buf[a, h, u, sl, :].astype(f32)
                    buf[a, h, u, sl, :] = (v * per_vreg[p]).astype(buf.dtype)

        def write(h, u0, nu):
            idx = (slice(None), pl.ds(h, 1), pl.ds(u0, nu))
            pltpu.make_async_copy(buf.at[idx], o_hbm.at[idx], write_sem).start()

        @pl.loop(0, units)
        def _(u):
            s = jax.nn.sigmoid(_tree_sum(wu_splat[u, r] * hidden[r] for r in range(rank)))
            s_ref[u] = s
            scale(0, u, s)
            write(0, u, 1)

        scales = [s_ref[u] for u in range(units)]

        @pl.loop(1, rows)
        def _(h):
            for u0 in range(0, units, _UNITS_PER_WRITE):
                for u in range(u0, u0 + _UNITS_PER_WRITE):
                    scale(h, u, scales[u])
                write(h, u0, _UNITS_PER_WRITE)

    pl.run_scoped(
        body,
        pltpu.SemaphoreType.DMA((len(reads),)),
        pltpu.SemaphoreType.DMA((2,)),
    )
    pltpu.make_async_copy(buf, o_hbm, write_sem).wait()


@jax.jit
def pallas_standalone__se_block__vision_kernel(
    x: jax.Array,
    w_down: jax.Array,
    w_up: jax.Array,
):
    batch, height, width, channels = x.shape
    rank = w_up.shape[0]
    units = channels // _PACKED
    w_tiles = width // _LANES
    rank_pad = pl.cdiv(rank, _SUBLANES) * _SUBLANES
    assert batch == 1 and height % _REGIONS == 0 and rank <= _LANES
    assert channels % (_PACKED * _UNITS_PER_WRITE) == 0 and width % _LANES == 0

    tiled = (height, channels // _SUBLANES, w_tiles, _SUBLANES, _LANES)
    view = (_REGIONS, height // _REGIONS, units, _PACKED * w_tiles, _LANES)
    x = x.reshape(height, w_tiles, _LANES, channels // _SUBLANES, _SUBLANES)
    x = x.transpose(0, 3, 1, 4, 2).reshape(view)

    out = pl.pallas_call(
        _se_kernel,
        in_specs=[pl.BlockSpec(memory_space=pltpu.HBM)] * 3,
        out_specs=pl.BlockSpec(memory_space=pltpu.HBM),
        out_shape=jax.ShapeDtypeStruct(view, x.dtype),
        scratch_shapes=[
            pltpu.VMEM(view, x.dtype),
            pltpu.VMEM((rank, channels), w_down.dtype),
            pltpu.VMEM((rank, channels), w_up.dtype),
            pltpu.VMEM((channels, _LANES), jnp.float32),
            pltpu.VMEM((_PACKED, rank_pad, _LANES), jnp.float32),
            pltpu.VMEM((units, rank, _PACKED, _LANES), jnp.float32),
            pltpu.VMEM((units, _PACKED, _LANES), jnp.float32),
            pltpu.SemaphoreType.DMA(()),
        ],
        compiler_params=pltpu.CompilerParams(vmem_limit_bytes=100 * 2**20),
    )(x, w_down.T, w_up)

    out = out.reshape(tiled).transpose(0, 2, 4, 1, 3)
    return out.reshape(batch, height, width, channels)
```

```python
import jax
import jax.numpy as jnp
from jax import lax
import jax.experimental.pallas as pl
import jax.experimental.pallas.tpu as pltpu

_LANES = 128
_SUBLANES = 8
_PACKED = 16

_REGIONS = 6
_UNITS_PER_WRITE = 3
_READ_REGIONS = (3, 2)
_READ_WIDE_ROWS = (19, 4, 1)
_READ_TAIL_ROWS = (20, 3, 1)


def _tree_sum(terms):
    terms = list(terms)
    while len(terms) > 1:
        terms = [
            terms[i] + terms[i + 1] if i + 1 < len(terms) else terms[i]
            for i in range(0, len(terms), 2)
        ]
    return terms[0]


def _read_plan(rows, units):
    last = _REGIONS - 1
    split = rows - sum(_READ_TAIL_ROWS)
    assert sum(_READ_REGIONS) == last and split > 0
    assert sum(_READ_WIDE_ROWS) == sum(_READ_TAIL_ROWS)
    head, tail = [], []
    a = 0
    for n in _READ_REGIONS:
        head.append((a, n, 0, rows, 0, units))
        a += n
    head.append((last, 1, 0, split, 0, units))
    h = split
    for n in _READ_WIDE_ROWS:
        head.append((last, 1, h, n, 0, units - 1))
        h += n
    h = split
    for n in _READ_TAIL_ROWS:
        tail.append((last, 1, h, n, units - 1, 1))
        h += n
    return head, tail


def _se_kernel(x_hbm, wd_hbm, wu_hbm, o_hbm,
               buf, wd_ref, wu_ref, wd_t, wd_splat, wu_splat, s_ref, write_sem):
    f32 = jnp.float32
    regions, rows, units, unit_rows, _ = buf.shape
    rank, channels = wu_ref.shape
    rank_pad = wd_splat.shape[1]
    vregs = unit_rows // _PACKED
    groups = 2 * units
    inv_n = 1.0 / (regions * rows * vregs * _LANES)
    head, tail = _read_plan(rows, units)
    reads = head + tail

    def groups_of(p):
        return (2 * p) // vregs, (2 * p + 1) // vregs

    def body(read_sems, weight_sems):
        def read(i):
            a0, na, h0, nh, u0, nu = reads[i]
            idx = (pl.ds(a0, na), pl.ds(h0, nh), pl.ds(u0, nu))
            return pltpu.make_async_copy(x_hbm.at[idx], buf.at[idx], read_sems.at[i])

        for i in range(len(reads)):
            read(i).start(priority=1)
        wd_copy = pltpu.make_async_copy(wd_hbm, wd_ref, weight_sems.at[0])
        wu_copy = pltpu.make_async_copy(wu_hbm, wu_ref, weight_sems.at[1])
        wd_copy.start()
        wu_copy.start()
        wd_copy.wait()
        wu_copy.wait()

        eye = (
            lax.broadcasted_iota(jnp.int32, (channels, channels), 0)
            == lax.broadcasted_iota(jnp.int32, (channels, channels), 1)
        ).astype(wd_ref.dtype)

        def transposed(w_ref):
            return lax.dot_general(
                eye, w_ref[...], (((1,), (1,)), ((), ())), preferred_element_type=f32
            )

        wd_t[...] = jnp.zeros_like(wd_t)
        wd_t[:, 0:rank] = transposed(wd_ref) * inv_n
        wd_splat[...] = jnp.zeros_like(wd_splat)
        wd = wd_ref[...].astype(f32) * inv_n
        for k in range(_PACKED):
            c = channels - _PACKED + k
            wd_splat[k, 0:rank, :] = jnp.broadcast_to(wd[:, c:c + 1], (rank, _LANES))
        wu_t = transposed(wu_ref)
        for r in range(rank):
            column = jnp.broadcast_to(wu_t[:, r:r + 1], (channels, _LANES))
            wu_splat[:, r] = column.reshape(units, _PACKED, _LANES)

        def add_units(acc, a, h, u0, nu):
            acc = dict(acc)
            for u in range(u0, u0 + nu):
                for p in range(vregs):
                    v = buf[a, h, u, pl.ds(_PACKED * p, _PACKED), :].astype(f32)
                    lo, hi = groups_of(p)
                    acc[2 * u + lo] += v[:_SUBLANES]
                    acc[2 * u + hi] += v[_SUBLANES:]
            return acc

        def consume(acc, i):
            a0, na, h0, nh, u0, nu = reads[i]
            step = min(nh, max(units // nu, 1))
            while nh % step:
                step -= 1

            def region(a, acc):
                def chunk(j, acc):
                    for k in range(step):
                        acc = add_units(acc, a, h0 + j * step + k, u0, nu)
                    return acc

                if nh == step:
                    return chunk(0, acc)
                return lax.fori_loop(0, nh // step, chunk, acc)

            read(i).wait()
            if na == 1:
                return region(a0, acc)
            return lax.fori_loop(a0, a0 + na, region, acc)

        acc = {g: jnp.zeros((_SUBLANES, _LANES), f32) for g in range(groups)}
        for i in range(len(head)):
            acc = consume(acc, i)

        z = _tree_sum(
            jnp.sum(acc[g], axis=1, keepdims=True) * wd_t[pl.ds(_SUBLANES * g, _SUBLANES), :]
            for g in range(groups - 2)
        )
        z = jnp.sum(z, axis=0, keepdims=True)
        diagonal = lax.broadcasted_iota(
            jnp.int32, (rank_pad, _LANES), 0
        ) == lax.broadcasted_iota(jnp.int32, (rank_pad, _LANES), 1)
        z = jnp.sum(jnp.where(diagonal, z, 0.0), axis=1, keepdims=True)
        z = jnp.broadcast_to(z, (rank_pad, _LANES))

        acc = {g: acc[g] for g in (groups - 2, groups - 1)}
        for i in range(len(head), len(reads)):
            acc = consume(acc, i)

        sums = jnp.concatenate([acc[groups - 2], acc[groups - 1]], axis=0)
        sums = jnp.broadcast_to(jnp.sum(sums, axis=1, keepdims=True), (_PACKED, _LANES))
        terms = [
            wd_splat[k] * jnp.broadcast_to(sums[k:k + 1, :], (rank_pad, _LANES))
            for k in range(_PACKED)
        ]
        terms[0] = terms[0] + z
        z = _tree_sum(terms)
        hidden = z * jax.nn.sigmoid(z)
        hidden = [
            jnp.broadcast_to(hidden[r:r + 1, :], (_PACKED, _LANES)) for r in range(rank)
        ]

        def scale_and_write(a0, na, h, u0, unit_scales):
            for k, s in enumerate(unit_scales):
                halves = (s[:_SUBLANES], s[_SUBLANES:])
                vreg_scales = [
                    jnp.concatenate([halves[g] for g in groups_of(p)], axis=0)
                    for p in range(vregs)
                ]
                for a in range(a0, a0 + na):
                    for p in range(vregs):
                        at = (a, h, u0 + k, pl.ds(_PACKED * p, _PACKED), slice(None))
                        buf[at] = (buf[at].astype(f32) * vreg_scales[p]).astype(buf.dtype)
            idx = (pl.ds(a0, na), pl.ds(h, 1), pl.ds(u0, len(unit_scales)))
            pltpu.make_async_copy(buf.at[idx], o_hbm.at[idx], write_sem).start()

        @pl.loop(0, units)
        def _(u):
            s = jax.nn.sigmoid(_tree_sum(wu_splat[u, r] * hidden[r] for r in range(rank)))
            s_ref[u] = s
            scale_and_write(0, 1, 0, u, [s])
            scale_and_write(1, regions - 1, 0, u, [s])

        scales = [s_ref[u] for u in range(units)]

        @pl.loop(1, rows)
        def _(h):
            for u0 in range(0, units, _UNITS_PER_WRITE):
                scale_and_write(0, regions, h, u0, scales[u0:u0 + _UNITS_PER_WRITE])

    pl.run_scoped(
        body,
        pltpu.SemaphoreType.DMA((len(reads),)),
        pltpu.SemaphoreType.DMA((2,)),
    )
    pltpu.make_async_copy(buf, o_hbm, write_sem).wait()


@jax.jit
def pallas_standalone__se_block__vision_kernel(
    x: jax.Array,
    w_down: jax.Array,
    w_up: jax.Array,
):
    batch, height, width, channels = x.shape
    rank = w_up.shape[0]
    units = channels // _PACKED
    w_tiles = width // _LANES
    rank_pad = pl.cdiv(rank, _SUBLANES) * _SUBLANES
    assert batch == 1 and height % _REGIONS == 0 and rank <= _LANES
    assert channels % (_PACKED * _UNITS_PER_WRITE) == 0 and width % _LANES == 0

    tiled = (height, channels // _SUBLANES, w_tiles, _SUBLANES, _LANES)
    view = (_REGIONS, height // _REGIONS, units, _PACKED * w_tiles, _LANES)
    x = x.reshape(height, w_tiles, _LANES, channels // _SUBLANES, _SUBLANES)
    x = x.transpose(0, 3, 1, 4, 2).reshape(view)

    out = pl.pallas_call(
        _se_kernel,
        in_specs=[pl.BlockSpec(memory_space=pltpu.HBM)] * 3,
        out_specs=pl.BlockSpec(memory_space=pltpu.HBM),
        out_shape=jax.ShapeDtypeStruct(view, x.dtype),
        scratch_shapes=[
            pltpu.VMEM(view, x.dtype),
            pltpu.VMEM((rank, channels), w_down.dtype),
            pltpu.VMEM((rank, channels), w_up.dtype),
            pltpu.VMEM((channels, _LANES), jnp.float32),
            pltpu.VMEM((_PACKED, rank_pad, _LANES), jnp.float32),
            pltpu.VMEM((units, rank, _PACKED, _LANES), jnp.float32),
            pltpu.VMEM((units, _PACKED, _LANES), jnp.float32),
            pltpu.SemaphoreType.DMA(()),
        ],
        compiler_params=pltpu.CompilerParams(vmem_limit_bytes=100 * 2**20),
    )(x, w_down.T, w_up)

    out = out.reshape(tiled).transpose(0, 2, 4, 1, 3)
    return out.reshape(batch, height, width, channels)
```
